```python
import jax
import jax.numpy as jnp

def _softmax(x, axis=-1):
    return jax.nn.softmax(x, axis=axis)
def _gelu(x):
    return jax.nn.gelu(x, approximate=True)
def _silu(x):
    return jax.nn.silu(x)
def _sigmoid(x):
    return jax.nn.sigmoid(x)
def _layernorm(x, axis=-1, eps=1e-5):
    m = jnp.mean(x, axis=axis, keepdims=True)
    v = jnp.var(x, axis=axis, keepdims=True)
    return (x - m) / jnp.sqrt(v + eps)
def _scatter_add(tgt, idx, src, axis=0):
    return tgt.at[idx].add(src)
def _segment_sum(src, seg, n):
    return jax.ops.segment_sum(src, seg, n)
class _Rng:
    def __init__(self, key):
        self._k = key
    def _next(self):
        self._k, sub = jax.random.split(self._k)
        return sub
    def normal(self, shape):
        return jax.random.normal(self._next(), shape, dtype=jnp.bfloat16)
    def randint(self, lo, hi, shape):
        return jax.random.randint(self._next(), shape, lo, hi, dtype=jnp.int32)
    def uniform(self, shape, lo=0.0, hi=1.0):
        return jax.random.uniform(self._next(), shape, jnp.bfloat16, lo, hi)
    def permutation(self, n):
        return jax.random.permutation(self._next(), n)


kernel_name = 'standalone__modern_conv_block_replknet__vision'

def setup_inputs():
    _rng = _Rng(jax.random.key(int.from_bytes(__import__("os").urandom(4), "little")))
    _w = (lambda a: (lambda t: t.astype(jnp.bfloat16) if jnp.issubdtype(t.dtype, jnp.floating) else t)(jnp.asarray(a)))
    H = W = 512
    C = 96
    K = 3
    return {
        "x": _w((lambda *s: _rng.normal(s) * 0.05)(1, H, W, C)),
        "dw_large": _w((lambda *s: _rng.normal(s) * 0.05)(K, K, C) * (1.0 / K)),
        "dw_small": _w((lambda *s: _rng.normal(s) * 0.05)(5, 5, C) * 0.2),
        "w1": _w((lambda *s: _rng.normal(s) * 0.05)(C, 4 * C) * (C ** -0.5)),
        "w2": _w((lambda *s: _rng.normal(s) * 0.05)(4 * C, C) * ((4 * C) ** -0.5)),
    }

def reference(x, dw_large, dw_small, w1, w2):
    B, H, W, C = x.shape
    Kl = dw_large.shape[0]
    pl = (Kl - 1) // 2
    xpl = jnp.pad(x, ((0,0),(pl,pl),(pl,pl),(0,0)))
    out = jnp.zeros_like(x)
    for i in range(Kl):
        for j in range(Kl):
            out = out + xpl[:, i:i+H, j:j+W, :] * dw_large[i, j][None, None, None, :]
    Ks = dw_small.shape[0]
    ps = (Ks - 1) // 2
    xps = jnp.pad(x, ((0,0),(ps,ps),(ps,ps),(0,0)))
    for i in range(Ks):
        for j in range(Ks):
            out = out + xps[:, i:i+H, j:j+W, :] * dw_small[i, j][None, None, None, :]
    h = _layernorm(out, axis=-1)
    h = _gelu(jnp.einsum('bhwc,ce->bhwe', h, w1))
    h = jnp.einsum('bhwe,ec->bhwc', h, w2)
    return x + h
```

```python
import functools
import math

import jax
import jax.numpy as jnp
import jax.experimental.pallas as pl
import jax.experimental.pallas.tpu as pltpu
from jax import lax

TH = 16
_A0 = math.sqrt(2.0 / math.pi)
_B0 = _A0 * 0.044715
_LAM = _B0 ** (1.0 / 3.0)
_A1 = _A0 / _LAM
_OUT_SCALE = 1.0 / (2.0 * _LAM)
_EPS = 1e-5


def _kernel(xm_ref, xt_ref, xb_ref, dwl_ref, dws_ref, w1_ref, w2t_ref, o_ref,
            kb_ref, w1t_ref, cv_ref, *, th, nblk):
    i = pl.program_id(0)
    C, W = xm_ref.shape[1], xm_ref.shape[2]
    f32 = jnp.float32

    @pl.when(i == 0)
    def _init():
        ks = dws_ref[...].astype(f32)
        kl = dwl_ref[...].astype(f32)
        rr = lax.broadcasted_iota(jnp.int32, (C, C), 0)
        cc = lax.broadcasted_iota(jnp.int32, (C, C), 1)
        for a in range(5):
            for b in range(5):
                k = ks[a, b:b + 1, :]
                if 1 <= a <= 3 and 1 <= b <= 3:
                    k = k + kl[a - 1, b - 1:b, :]
                col = jnp.sum(jnp.where(rr == cc, jnp.broadcast_to(k, (C, C)), 0.0),
                              axis=1, keepdims=True)
                kb_ref[a * 5 + b] = jnp.broadcast_to(col, (C, 128))
        w1t_ref[...] = w1_ref[...].astype(f32).T.astype(jnp.bfloat16)

    lane = lax.broadcasted_iota(jnp.int32, (8, W), 1)
    top_ok = i > 0
    bot_ok = i < nblk - 1

    def conv_group(g, carry):
        c0 = pl.multiple_of(g * 16, 16)
        acc = {}
        for r in range(-2, th + 2):
            if r < 0:
                xr = xt_ref[r + 2, pl.ds(c0, 16), :]
            elif r >= th:
                xr = xb_ref[r - th, pl.ds(c0, 16), :]
            else:
                xr = xm_ref[r, pl.ds(c0, 16), :]
            xr = xr.astype(f32)
            if r < 0:
                xr = jnp.where(top_ok, xr, 0.0)
            elif r >= th:
                xr = jnp.where(bot_ok, xr, 0.0)
            for half in range(2):
                v = xr[half * 8:(half + 1) * 8]
                for b in range(5):
                    s = b - 2
                    if s == 0:
                        vs = v
                    elif s < 0:
                        vs = jnp.where(lane >= -s, pltpu.roll(v, -s, 1), 0.0)
                    else:
                        vs = jnp.where(lane < W - s, pltpu.roll(v, W - s, 1), 0.0)
                    for a in range(5):
                        ro = r - (a - 2)
                        if ro < 0 or ro >= th:
                            continue
                        k = kb_ref[a * 5 + b, pl.ds(c0 + half * 8, 8), :]
                        k = jnp.concatenate([k] * (W // 128), axis=1)
                        t = vs * k
                        key = (ro, half)
                        acc[key] = t if key not in acc else acc[key] + t
                ro = r - 2
                if 0 <= ro < th:
                    cv_ref[ro, pl.ds(c0 + half * 8, 8), :] = acc.pop((ro, half))
        return carry

    lax.fori_loop(0, C // 16, conv_group, 0)

    def mlp_row(r, carry):
        y = cv_ref[r]
        m = jnp.sum(y, axis=0, keepdims=True) * (1.0 / C)
        d = y - m
        var = jnp.sum(d * d, axis=0, keepdims=True) * (1.0 / C)
        hn = (d * (lax.rsqrt(var + _EPS) * _LAM)).astype(jnp.bfloat16)
        a = jnp.dot(w1t_ref[...], hn, preferred_element_type=f32)
        g = (a * (1.0 + jnp.tanh(a * (a * a + _A1)))).astype(jnp.bfloat16)
        o = jnp.dot(w2t_ref[...], g, preferred_element_type=f32)
        o_ref[r] = (xm_ref[r].astype(f32) + o * _OUT_SCALE).astype(o_ref.dtype)
        return carry

    lax.fori_loop(0, th, mlp_row, 0, unroll=2)


@jax.jit
def pallas_standalone__modern_conv_block_replknet__vision_kernel(
    x: jax.Array,
    dw_large: jax.Array,
    dw_small: jax.Array,
    w1: jax.Array,
    w2: jax.Array,
):
    B, H, W, C = x.shape
    E = w1.shape[1]
    th = TH
    nblk = H // th
    xt = jnp.transpose(x, (0, 1, 3, 2)).reshape(H, C, W)
    w2t = w2.T
    hb = th // 2
    out = pl.pallas_call(
        functools.partial(_kernel, th=th, nblk=nblk),
        grid=(nblk,),
        in_specs=[
            pl.BlockSpec((th, C, W), lambda i: (i, 0, 0)),
            pl.BlockSpec((2, C, W), lambda i: (jnp.maximum(i * hb - 1, 0), 0, 0)),
            pl.BlockSpec((2, C, W), lambda i: (jnp.minimum((i + 1) * hb, H // 2 - 1), 0, 0)),
            pl.BlockSpec(dw_large.shape, lambda i: (0, 0, 0)),
            pl.BlockSpec(dw_small.shape, lambda i: (0, 0, 0)),
            pl.BlockSpec(w1.shape, lambda i: (0, 0)),
            pl.BlockSpec(w2t.shape, lambda i: (0, 0)),
        ],
        out_specs=pl.BlockSpec((th, C, W), lambda i: (i, 0, 0)),
        out_shape=jax.ShapeDtypeStruct((H, C, W), x.dtype),
        scratch_shapes=[
            pltpu.VMEM((25, C, 128), jnp.float32),
            pltpu.VMEM((E, C), jnp.bfloat16),
            pltpu.VMEM((th, C, W), jnp.float32),
        ],
        compiler_params=pltpu.CompilerParams(
            dimension_semantics=("arbitrary",),
            vmem_limit_bytes=64 * 1024 * 1024,
        ),
    )(xt, xt, xt, dw_large, dw_small, w1, w2t)
    return jnp.transpose(out.reshape(B, H, C, W), (0, 1, 3, 2))
```

```python
import functools
import math

import jax
import jax.numpy as jnp
import jax.experimental.pallas as pl
import jax.experimental.pallas.tpu as pltpu
from jax import lax

TH = 8
U = 1
NW = 512
ME = 128
_A0 = math.sqrt(2.0 / math.pi)
_B0 = _A0 * 0.044715
_LAM = _B0 ** (1.0 / 3.0)
_A1 = _A0 / _LAM
_OUT_SCALE = 1.0 / (2.0 * _LAM)
_EPS = 1e-5


def _perm(p):
    return (p // 16) * 16 + 2 * (p % 8) + (p % 16) // 8


def _kernel(xm_ref, xr_ref, dwl_ref, dws_ref, w1_ref, w2t_ref, o_ref,
            kb_ref, w1t_ref, cv_ref, acc_ref, un_ref, hn_ref, g_ref, *, th, nblk):
    i = pl.program_id(0)
    C, W = xm_ref.shape[1], xm_ref.shape[2]
    NT = W // 128
    f32 = jnp.float32

    @pl.when(i == 0)
    def _init():
        ks = dws_ref[...].astype(f32)
        kl = dwl_ref[...].astype(f32)
        rr = lax.broadcasted_iota(jnp.int32, (C, C), 0)
        cc = lax.broadcasted_iota(jnp.int32, (C, C), 1)
        sel = _perm(rr) == cc
        for a in range(5):
            for b in range(5):
                k = ks[a, b:b + 1, :]
                if 1 <= a <= 3 and 1 <= b <= 3:
                    k = k + kl[a - 1, b - 1:b, :]
                col = jnp.sum(jnp.where(sel, jnp.broadcast_to(k, (C, C)), 0.0),
                              axis=1, keepdims=True)
                kb_ref[a * 5 + b] = jnp.broadcast_to(col, (C, 128))
        w1p = jnp.dot(jnp.where(sel, 1.0, 0.0).astype(jnp.bfloat16), w1_ref[...],
                      preferred_element_type=f32)
        w1t_ref[...] = w1p.T.astype(jnp.bfloat16)
        cv_ref[...] = jnp.zeros(cv_ref.shape, f32)
        acc_ref[...] = jnp.zeros(acc_ref.shape, f32)
        hn_ref[...] = jnp.zeros(hn_ref.shape, hn_ref.dtype)
        g_ref[...] = jnp.zeros(g_ref.shape, g_ref.dtype)
        un_ref[0] = jnp.full((8, 128), 16, jnp.uint32)
        un_ref[1] = jnp.full((8, 128), 0xFFFF0000, jnp.uint32)

    lane = lax.broadcasted_iota(jnp.int32, (8, 128), 1)
    row_ok = i < nblk

    def conv(r, c0, half):
        cs = pl.ds(c0 + half * 8, 8)
        acc = {(a, t): acc_ref[a - 1, cs, t * 128:(t + 1) * 128]
               for a in range(1, 5) for t in range(NT)}
        if True:
            wd = pltpu.bitcast(xm_ref[r, pl.ds(c0, 16), :], jnp.uint32)
            un = un_ref[half]
            vt = []
            for t in range(NT):
                u = wd[:, t * 128:(t + 1) * 128]
                u = (u << un) if half == 0 else (u & un)
                vt.append(jnp.where(row_ok, pltpu.bitcast(u, f32), 0.0))
            for b in range(5):
                s = b - 2
                if s == 0:
                    vs = vt
                elif s < 0:
                    ro = [pltpu.roll(u, -s, 1) for u in vt]
                    vs = [jnp.where(lane >= -s, ro[t], ro[t - 1] if t > 0 else 0.0)
                          for t in range(NT)]
                else:
                    ro = [pltpu.roll(u, 128 - s, 1) for u in vt]
                    vs = [jnp.where(lane < 128 - s, ro[t], ro[t + 1] if t < NT - 1 else 0.0)
                          for t in range(NT)]
                for a in range(5):
                    k = kb_ref[a * 5 + b, cs, :]
                    for t in range(NT):
                        p = vs[t] * k
                        key = (a, t)
                        acc[key] = p if key not in acc else acc[key] + p
                yield
            for a in range(4):
                acc_ref[a, cs, :] = jnp.concatenate([acc[(a, t)] for t in range(NT)], axis=1)
            cv_ref[(i * th + r + 2 * th - 2) % (2 * th), cs, :] = jnp.concatenate(
                [acc[(4, t)] for t in range(NT)], axis=1)
            yield

    def mlp(r, n0):
        ls = slice(n0, n0 + NW)
        o = jnp.dot(w2t_ref[...], g_ref[:, ls], preferred_element_type=f32)
        o_ref[r, :, ls] = (xr_ref[r, :, ls].astype(f32) + o * _OUT_SCALE).astype(o_ref.dtype)
        yield
        for e in range(0, w1t_ref.shape[0], ME):
            a = jnp.dot(w1t_ref[e:e + ME, :], hn_ref[:, ls], preferred_element_type=f32)
            g_ref[e:e + ME, ls] = (a * (1.0 + jnp.tanh(a * (a * a + _A1)))).astype(jnp.bfloat16)
            yield
        y = cv_ref[(i * th + r + th + 2) % (2 * th), :, ls]
        m = jnp.sum(y, axis=0, keepdims=True) * (1.0 / C)
        d = y - m
        var = jnp.sum(d * d, axis=0, keepdims=True) * (1.0 / C)
        hn_ref[:, ls] = (d * (lax.rsqrt(var + _EPS) * _LAM)).astype(jnp.bfloat16)
        yield

    def body(j, carry):
        def chain(gens):
            for g in gens:
                yield from g
        cg = chain([conv(j * U + u, q * 16, hf) for u in range(U) for q in range(C // 16) for hf in range(2)])
        mg = chain([mlp(j * U + q, n0) for q in range(U) for n0 in range(0, W, NW)])
        nc = U * (C // 8) * 6
        nm = U * (W // NW) * (2 + w1t_ref.shape[0] // ME)
        dc = dm = 0
        while dc < nc or dm < nm:
            if dm >= nm or (dc < nc and dc * nm <= dm * nc):
                next(cg)
                dc += 1
            else:
                next(mg)
                dm += 1
        return carry

    lax.fori_loop(0, th // U, body, 0)


@jax.jit
def pallas_standalone__modern_conv_block_replknet__vision_kernel(
    x: jax.Array,
    dw_large: jax.Array,
    dw_small: jax.Array,
    w1: jax.Array,
    w2: jax.Array,
):
    B, H, W, C = x.shape
    E = w1.shape[1]
    th = TH
    nblk = H // th
    xt = jnp.transpose(x, (0, 1, 3, 2)).reshape(H, C, W)
    w2t = w2.T
    out = pl.pallas_call(
        functools.partial(_kernel, th=th, nblk=nblk),
        grid=(nblk + 1,),
        in_specs=[
            pl.BlockSpec((th, C, W), lambda i: (jnp.minimum(i, nblk - 1), 0, 0)),
            pl.BlockSpec((th, C, W), lambda i: (jnp.maximum(i - 1, 0), 0, 0)),
            pl.BlockSpec(dw_large.shape, lambda i: (0, 0, 0)),
            pl.BlockSpec(dw_small.shape, lambda i: (0, 0, 0)),
            pl.BlockSpec(w1.shape, lambda i: (0, 0)),
            pl.BlockSpec(w2t.shape, lambda i: (0, 0)),
        ],
        out_specs=pl.BlockSpec((th, C, W), lambda i: (jnp.maximum(i - 1, 0), 0, 0)),
        out_shape=jax.ShapeDtypeStruct((H, C, W), x.dtype),
        scratch_shapes=[
            pltpu.VMEM((25, C, 128), jnp.float32),
            pltpu.VMEM((E, C), jnp.bfloat16),
            pltpu.VMEM((2 * th, C, W), jnp.float32),
            pltpu.VMEM((4, C, W), jnp.float32),
            pltpu.VMEM((2, 8, 128), jnp.uint32),
            pltpu.VMEM((C, W), jnp.bfloat16),
            pltpu.VMEM((E, W), jnp.bfloat16),
        ],
        compiler_params=pltpu.CompilerParams(
            dimension_semantics=("arbitrary",),
            vmem_limit_bytes=64 * 1024 * 1024,
        ),
    )(xt, xt, dw_large, dw_small, w1, w2t)
    return jnp.transpose(out.reshape(B, H, C, W), (0, 1, 3, 2))
```
